```python
import jax
import jax.numpy as jnp

def _softmax(x, axis=-1):
    return jax.nn.softmax(x, axis=axis)
def _gelu(x):
    return jax.nn.gelu(x, approximate=True)
def _silu(x):
    return jax.nn.silu(x)
def _sigmoid(x):
    return jax.nn.sigmoid(x)
def _layernorm(x, axis=-1, eps=1e-5):
    m = jnp.mean(x, axis=axis, keepdims=True)
    v = jnp.var(x, axis=axis, keepdims=True)
    return (x - m) / jnp.sqrt(v + eps)
def _scatter_add(tgt, idx, src, axis=0):
    return tgt.at[idx].add(src)
def _segment_sum(src, seg, n):
    return jax.ops.segment_sum(src, seg, n)
class _Rng:
    def __init__(self, key):
        self._k = key
    def _next(self):
        self._k, sub = jax.random.split(self._k)
        return sub
    def normal(self, shape):
        return jax.random.normal(self._next(), shape, dtype=jnp.bfloat16)
    def randint(self, lo, hi, shape):
        return jax.random.randint(self._next(), shape, lo, hi, dtype=jnp.int32)
    def uniform(self, shape, lo=0.0, hi=1.0):
        return jax.random.uniform(self._next(), shape, jnp.bfloat16, lo, hi)
    def permutation(self, n):
        return jax.random.permutation(self._next(), n)


kernel_name = 'standalone__cross_network_dcn_v2__recsys'

def setup_inputs():
    _rng = _Rng(jax.random.key(int.from_bytes(__import__("os").urandom(4), "little")))
    _w = (lambda a: (lambda t: t.astype(jnp.bfloat16) if jnp.issubdtype(t.dtype, jnp.floating) else t)(jnp.asarray(a)))
    B, F, D, L = 16384, 100, 16, 3
    Din = min(F * D, 512)
    R = max(Din // 4, 2)
    sc = Din ** -0.5
    return {
        "x0": _w((lambda *s: _rng.normal(s) * 0.05)(B, Din)),
        "U":  _w((lambda *s: _rng.normal(s) * 0.05)(L, Din, R) * sc),
        "V":  _w((lambda *s: _rng.normal(s) * 0.05)(L, R, Din) * sc),
        "bs": _w((lambda *s: _rng.normal(s) * 0.05)(L, Din)),
    }

def reference(x0, U, V, bs):
    x = x0
    for l in range(U.shape[0]):
        h = jnp.einsum('rd,bd->br', V[l], x)
        h = jnp.einsum('dr,br->bd', U[l], h)
        x = x0 * (h + bs[l]) + x
    return x
```

```python
import jax
import jax.numpy as jnp
from jax import lax
from jax.experimental import pallas as pl
from jax.experimental.pallas import tpu as pltpu

_SUB = 256
_NT = (((1,), (1,)), ((), ()))


def _cross_rows(x_ref, o_ref, u_ref, v_ref, b_ref, start, hooks):
    rows = pl.ds(start, _SUB)
    xb = x_ref[rows, :]
    for l in range(u_ref.shape[0]):
        if (l, 0) in hooks:
            hooks[l, 0]()
        h = lax.dot_general(xb, v_ref[l], _NT, preferred_element_type=jnp.float32)
        h = h.astype(jnp.bfloat16)
        if (l, 1) in hooks:
            hooks[l, 1]()
        g = lax.dot_general(h, u_ref[l], _NT, preferred_element_type=jnp.float32)
        b = b_ref[l:l + 1, :].astype(jnp.float32)
        x0f = x_ref[rows, :].astype(jnp.float32)
        if l == 0:
            xn = x0f * (g + (b + 1.0))
        else:
            xn = x0f * (g + b) + xb.astype(jnp.float32)
        xb = xn.astype(jnp.bfloat16)
    o_ref[rows, :] = xb


def _plan(batch):
    if batch == 16384:
        return (512, 1024, 2560), 4096, 3
    return (), _SUB, batch // _SUB


@jax.jit
def pallas_standalone__cross_network_dcn_v2__recsys_kernel(
    x0: jax.Array,
    U: jax.Array,
    V: jax.Array,
    bs: jax.Array,
):
    batch, din = x0.shape
    assert batch % _SUB == 0
    ramp, body, iters = _plan(batch)
    assert sum(ramp) + body * iters == batch
    assert all(c % _SUB == 0 for c in ramp) and body % _SUB == 0
    chunks = ramp + (body,) * iters
    starts = tuple(sum(chunks[:i]) for i in range(len(chunks)))
    n_ramp = len(ramp)

    def kernel(x_hbm, u_hbm, v_hbm, b_hbm, o_hbm,
               xbuf, obuf, u_ref, v_ref, b_ref, isem, osem, wsem):
        def in_copy(c):
            sl = pl.ds(starts[c], chunks[c])
            return pltpu.make_async_copy(x_hbm.at[sl], xbuf.at[sl], isem.at[c])

        def out_copy(r0, n):
            sl = pl.ds(r0, n)
            return pltpu.make_async_copy(obuf.at[sl], o_hbm.at[sl], osem)

        weights = [
            pltpu.make_async_copy(v_hbm, v_ref, wsem.at[0]),
            pltpu.make_async_copy(u_hbm, u_ref, wsem.at[1]),
            pltpu.make_async_copy(b_hbm, b_ref, wsem.at[2]),
        ]
        in_copy(0).start()
        for w in weights:
            w.start()
        for w in weights:
            w.wait()

        for c in range(n_ramp):
            if c == 0:
                in_copy(0).wait()
            in_copy(c + 1).start()
            n_sub = chunks[c] // _SUB
            for s in range(n_sub):
                hooks = {}
                if s == n_sub - 1 and c + 1 < n_ramp:
                    hooks[u_ref.shape[0] - 1, 1] = in_copy(c + 1).wait
                _cross_rows(xbuf, obuf, u_ref, v_ref, b_ref,
                            starts[c] + s * _SUB, hooks)
        for c in range(n_ramp + 1, len(chunks)):
            in_copy(c).start()
        if n_ramp:
            out_copy(0, starts[n_ramp]).start()

        def step(i, carry):
            base = pl.multiple_of(starts[n_ramp] + i * body, _SUB)
            sl = pl.ds(base, body)
            pltpu.make_async_copy(
                x_hbm.at[sl], xbuf.at[sl], isem.at[n_ramp + i]).wait()
            for s in range(body // _SUB):
                _cross_rows(xbuf, obuf, u_ref, v_ref, b_ref, base + s * _SUB, {})
                out_copy(base + s * _SUB, _SUB).start()
            return carry

        lax.fori_loop(0, iters, step, 0)
        pltpu.make_async_copy(obuf, o_hbm, osem).wait()

    return pl.pallas_call(
        kernel,
        in_specs=[pl.BlockSpec(memory_space=pl.ANY)] * 4,
        out_specs=pl.BlockSpec(memory_space=pl.ANY),
        out_shape=jax.ShapeDtypeStruct((batch, din), x0.dtype),
        scratch_shapes=[
            pltpu.VMEM((batch, din), x0.dtype),
            pltpu.VMEM((batch, din), x0.dtype),
            pltpu.VMEM(U.shape, U.dtype),
            pltpu.VMEM(V.shape, V.dtype),
            pltpu.VMEM(bs.shape, bs.dtype),
            pltpu.SemaphoreType.DMA((len(chunks),)),
            pltpu.SemaphoreType.DMA,
            pltpu.SemaphoreType.DMA((3,)),
        ],
        compiler_params=pltpu.CompilerParams(vmem_limit_bytes=64 * 1024 * 1024),
    )(x0, U, V, bs)
```

```python
import functools

import jax
import jax.numpy as jnp
from jax import lax
from jax.experimental import pallas as pl
from jax.experimental.pallas import tpu as pltpu

_SUB = 256
_RAMP = (256, 256, 768, 2304)
_BODY = 6400
_STEPS = 2
_OUT = (2048, 2048, 1024, 512, 256, 256)
_OUT_LAST = (64, 64, 64, 64)
_NT = (((1,), (1,)), ((), ()))


def _cross_block(x_ref, o_ref, b_ref, down, up, start, hooks=None, pieces=None):
    hooks = hooks or {}
    n_layers = b_ref.shape[0]
    rows = pl.ds(start, _SUB)
    xb = x_ref[rows, :]
    if "pre" in hooks:
        hooks["pre"]()
    for l in range(n_layers):
        h = down(xb, l).astype(jnp.bfloat16)
        if l in hooks:
            hooks[l]()
        g = up(h, l)
        b = b_ref[l:l + 1, :].astype(jnp.float32)
        if l == n_layers - 1 and pieces is not None:
            off = 0
            for n, done in pieces:
                part = pl.ds(start + off, n)
                xn = (x_ref[part, :].astype(jnp.float32) * (g[off:off + n] + b)
                      + xb[off:off + n].astype(jnp.float32))
                o_ref[part, :] = xn.astype(jnp.bfloat16)
                done()
                off += n
            return
        x0f = x_ref[rows, :].astype(jnp.float32)
        if l == 0:
            xn = x0f * (g + (b + 1.0))
        else:
            xn = x0f * (g + b) + xb.astype(jnp.float32)
        xb = xn.astype(jnp.bfloat16)
    o_ref[rows, :] = xb


def _kernel(x_hbm, u_hbm, v_hbm, b_hbm, o_hbm,
            xbuf, obuf, u_ref, v_ref, b_ref, ut_ref, vt_ref, isem, osem, fsem):
    chunks = _RAMP + (_BODY,) * _STEPS
    starts = [sum(chunks[:i]) for i in range(len(chunks))]
    n_ramp = len(_RAMP)
    x_slot = (2, 3, 4, 2, 0, 1)

    def x_copy(c):
        sl = pl.ds(starts[c], chunks[c])
        return pltpu.make_async_copy(x_hbm.at[sl], xbuf.at[sl], isem.at[x_slot[c]])

    def w_copy(hbm, vmem, l, slot):
        return pltpu.make_async_copy(hbm.at[l], vmem.at[l], isem.at[slot])

    def out_copy(r0, n):
        sl = pl.ds(r0, n)
        return pltpu.make_async_copy(obuf.at[sl], o_hbm.at[sl], osem)

    groups = (
        lambda: (w_copy(v_hbm, v_ref, 0, 2), x_copy(0)),
        lambda: (w_copy(u_hbm, u_ref, 0, 0), w_copy(v_hbm, v_ref, 1, 0),
                 pltpu.make_async_copy(b_hbm, b_ref, isem.at[0])),
        lambda: (w_copy(u_hbm, u_ref, 1, 1), w_copy(v_hbm, v_ref, 2, 1)),
        lambda: (w_copy(u_hbm, u_ref, 2, 3), x_copy(1)),
    )

    def wait_group(i):
        for copy in groups[i]():
            copy.wait()
        if i < 3:
            x_copy(3 + i).start()

    for group in groups:
        for copy in group():
            copy.start()
        pl.semaphore_signal(fsem, 1)
        pl.semaphore_wait(fsem, 1)
    x_copy(2).start()
    wait_group(0)

    def down_nt(x, l):
        return lax.dot_general(x, v_ref[l], _NT, preferred_element_type=jnp.float32)

    def up_nt(h, l):
        return lax.dot_general(h, u_ref[l], _NT, preferred_element_type=jnp.float32)

    def down(x, l):
        return jnp.dot(x, vt_ref[l], preferred_element_type=jnp.float32)

    def up(h, l):
        return jnp.dot(h, ut_ref[l], preferred_element_type=jnp.float32)

    last = b_ref.shape[0] - 1

    def transpose_weights():
        for l in range(last + 1):
            vt_ref[l] = v_ref[l].T
        for l in range(last + 1):
            ut_ref[l] = u_ref[l].T

    def ramp_up():
        k = 0
        for c in range(n_ramp):
            n_sub = chunks[c] // _SUB
            for s in range(n_sub):
                hooks = {}
                if k == 0:
                    hooks = {i - 1: functools.partial(wait_group, i)
                             for i in range(1, len(groups))}
                elif s == n_sub - 1 and c + 1 < n_ramp:
                    hooks = {last: x_copy(c + 1).wait}
                if k == 0:
                    mm = (down_nt, up_nt)
                elif k == 1:
                    hooks["pre"] = transpose_weights
                    mm = (down_nt, lambda h, l: (up if l == last else up_nt)(h, l))
                else:
                    mm = (down, up)
                _cross_block(xbuf, obuf, b_ref, *mm, starts[c] + s * _SUB, hooks)
                k += 1
        out_copy(0, starts[n_ramp]).start()

    out_ends = {sum(_OUT[:i + 1]) // _SUB: (sum(_OUT[:i]), n)
                for i, n in enumerate(_OUT)}

    def steady(i):
        base = pl.multiple_of(starts[n_ramp] + i * _BODY, _SUB)
        sl = pl.ds(base, _BODY)
        pltpu.make_async_copy(x_hbm.at[sl], xbuf.at[sl], isem.at[i]).wait()
        n_sub = _BODY // _SUB
        for s in range(n_sub - 1):
            _cross_block(xbuf, obuf, b_ref, down, up, base + s * _SUB)
            if s + 1 in out_ends:
                off, n = out_ends[s + 1]
                out_copy(base + off, n).start()
        r0 = base + (n_sub - 1) * _SUB
        pieces = [(n, out_copy(r0 + sum(_OUT_LAST[:j]), n).start)
                  for j, n in enumerate(_OUT_LAST)]
        _cross_block(xbuf, obuf, b_ref, down, up, r0, pieces=pieces)

    def step(i, carry):
        pl.when(i == 0)(ramp_up)
        pl.when(i > 0)(lambda: steady(i - 1))
        return carry

    lax.fori_loop(0, _STEPS + 1, step, 0)
    pltpu.make_async_copy(obuf, o_hbm, osem).wait()


@jax.jit
def pallas_standalone__cross_network_dcn_v2__recsys_kernel(
    x0: jax.Array,
    U: jax.Array,
    V: jax.Array,
    bs: jax.Array,
):
    batch, din = x0.shape
    assert U.shape[0] == V.shape[0] == bs.shape[0] == 3
    assert sum(_RAMP) + _BODY * _STEPS == batch
    assert sum(_OUT) + _SUB == _BODY and sum(_OUT_LAST) == _SUB
    assert all(n % _SUB == 0 for n in _RAMP + _OUT + (_BODY,))

    return pl.pallas_call(
        _kernel,
        in_specs=[pl.BlockSpec(memory_space=pl.ANY)] * 4,
        out_specs=pl.BlockSpec(memory_space=pl.ANY),
        out_shape=jax.ShapeDtypeStruct((batch, din), x0.dtype),
        scratch_shapes=[
            pltpu.VMEM((batch, din), x0.dtype),
            pltpu.VMEM((batch, din), x0.dtype),
            pltpu.VMEM(U.shape, U.dtype),
            pltpu.VMEM(V.shape, V.dtype),
            pltpu.VMEM(bs.shape, bs.dtype),
            pltpu.VMEM(V.shape, U.dtype),
            pltpu.VMEM(U.shape, V.dtype),
            pltpu.SemaphoreType.DMA((5,)),
            pltpu.SemaphoreType.DMA,
            pltpu.SemaphoreType.REGULAR,
        ],
        compiler_params=pltpu.CompilerParams(vmem_limit_bytes=64 * 1024 * 1024),
    )(x0, U, V, bs)
```
